```python
import jax
import jax.numpy as jnp

def _softmax(x, axis=-1):
    return jax.nn.softmax(x, axis=axis)
def _gelu(x):
    return jax.nn.gelu(x, approximate=True)
def _silu(x):
    return jax.nn.silu(x)
def _sigmoid(x):
    return jax.nn.sigmoid(x)
def _layernorm(x, axis=-1, eps=1e-5):
    m = jnp.mean(x, axis=axis, keepdims=True)
    v = jnp.var(x, axis=axis, keepdims=True)
    return (x - m) / jnp.sqrt(v + eps)
def _scatter_add(tgt, idx, src, axis=0):
    return tgt.at[idx].add(src)
def _segment_sum(src, seg, n):
    return jax.ops.segment_sum(src, seg, n)
class _Rng:
    def __init__(self, key):
        self._k = key
    def _next(self):
        self._k, sub = jax.random.split(self._k)
        return sub
    def normal(self, shape):
        return jax.random.normal(self._next(), shape, dtype=jnp.bfloat16)
    def randint(self, lo, hi, shape):
        return jax.random.randint(self._next(), shape, lo, hi, dtype=jnp.int32)
    def uniform(self, shape, lo=0.0, hi=1.0):
        return jax.random.uniform(self._next(), shape, jnp.bfloat16, lo, hi)
    def permutation(self, n):
        return jax.random.permutation(self._next(), n)


kernel_name = 'concat_heads__mha_block_cached__compressed_kv_cla__decode'

def setup_inputs():
    _rng = _Rng(jax.random.key(int.from_bytes(__import__("os").urandom(4), "little")))
    _w = (lambda a: (lambda t: t.astype(jnp.bfloat16) if jnp.issubdtype(t.dtype, jnp.floating) else t)(jnp.asarray(a)))
    def _A_setup():
        B, Sq, D = 4, 1, 576
        H, Sk, Dh = 32, 4096, 128
        return {
            "x": _w((lambda *s: _rng.normal(s) * 0.05)(B, Sq, D)),
            "k_cache": _w((lambda *s: _rng.normal(s) * 0.05)(B, H, Sk, Dh)),
            "v_cache": _w((lambda *s: _rng.normal(s) * 0.05)(B, H, Sk, Dh)),
            "wq": _w((lambda *s: _rng.normal(s) * 0.05)(D, H * Dh) * (D ** -0.5)),
            "wo": _w((lambda *s: _rng.normal(s) * 0.05)(H * Dh, D) * ((H * Dh) ** -0.5)),
        }
    _A_in = _A_setup()

    def _B_setup():
        B, H, Sq, Sk, D, M = 4, 32, 1, 4096, 128, 576
        Dc = 4 * D
        return {
            "x": _w((lambda *s: _rng.normal(s) * 0.05)(B, Sq, M)),
            "c_kv": _w((lambda *s: _rng.normal(s) * 0.05)(B, Sk, Dc)),
            "w_q": _w((lambda *s: _rng.normal(s) * 0.05)(M, H, D) * (M ** -0.5)),
            "w_uk": _w((lambda *s: _rng.normal(s) * 0.05)(Dc, H, D) * (Dc ** -0.5)),
            "w_uv": _w((lambda *s: _rng.normal(s) * 0.05)(Dc, H, D) * (Dc ** -0.5)),
            "w_o": _w((lambda *s: _rng.normal(s) * 0.05)(H, D, M) * ((H * D) ** -0.5)),
        }
    _B_in = _B_setup()

    return {
        "A_x": _A_in["x"],
        "A_k_cache": _A_in["k_cache"],
        "A_v_cache": _A_in["v_cache"],
        "A_wq": _A_in["wq"],
        "A_wo": _A_in["wo"],
        "B_x": _B_in["x"],
        "B_c_kv": _B_in["c_kv"],
        "B_w_q": _B_in["w_q"],
        "B_w_uk": _B_in["w_uk"],
        "B_w_uv": _B_in["w_uv"],
        "B_w_o": _B_in["w_o"],
    }

def reference(A_x, A_k_cache, A_v_cache, A_wq, A_wo, B_x, B_c_kv, B_w_q, B_w_uk, B_w_uv, B_w_o):
    def _A_ref(x, k_cache, v_cache, wq, wo):
        B, Sq, D = x.shape
        H, Dh = 32, 128
        q = (lambda x, *d: x.transpose(*d))((x @ wq).reshape(B, Sq, H, Dh), 0, 2, 1, 3)
        scores = jnp.einsum("bhqd,bhkd->bhqk", q, k_cache) * (Dh ** -0.5)
        p = _softmax(scores, axis=-1)
        o = jnp.einsum("bhqk,bhkd->bhqd", p, v_cache)
        return (lambda x, *d: x.transpose(*d))(o, 0, 2, 1, 3).reshape(B, Sq, H * Dh) @ wo

    def _B_ref(x, c_kv, w_q, w_uk, w_uv, w_o):
        B, Sq, M = x.shape[0], x.shape[1], x.shape[2]
        Sk = c_kv.shape[1]
        H, D = w_q.shape[1], w_q.shape[2]
        q = jnp.einsum("bqm,mhd->bhqd", x, w_q)
        k = jnp.einsum("bkc,chd->bhkd", c_kv, w_uk)
        v = jnp.einsum("bkc,chd->bhkd", c_kv, w_uv)
        scores = jnp.einsum("bhqd,bhkd->bhqk", q, k) * (D ** -0.5)
        off = Sk - Sq
        qi = jnp.arange(Sq)[:, None]
        kj = jnp.arange(Sk)[None, :]
        cmask = kj <= (qi + off)
        scores = jnp.where(cmask[None, None], scores, -1e9)
        p = _softmax(scores, axis=-1)
        ctx = jnp.einsum("bhqk,bhkd->bhqd", p, v)
        return jnp.einsum("bhqd,hdm->bqm", ctx, w_o)

    a = _A_ref(A_x, A_k_cache, A_v_cache, A_wq, A_wo)
    b = _B_ref(B_x, B_c_kv, B_w_q, B_w_uk, B_w_uv, B_w_o)
    return jnp.concatenate([a, b], axis=-1)
```

```python
import jax
import jax.numpy as jnp
from jax import lax
import jax.experimental.pallas as pl
import jax.experimental.pallas.tpu as pltpu

_B, _H, _S, _D, _M, _C = 4, 32, 4096, 128, 576, 512
_NT = (((1,), (1,)), ((), ()))
F32, BF16 = jnp.float32, jnp.bfloat16


def _make(nbuf=4, skip_dma=False):
    def body(xa_h, k_h, v_h, wq_h, wo_h, xb_h, c_h, bwq_h, wuk_h, wuv_h, bwo_h, o_ref,
             xa_v, xb_v, wq_v, wo_v, c_v, bwq_v, wuk_v, wuv_v, bwo_v, k_v, v_v, qa_s, oa_s, qc_s, cc_s, wsem, ksem, vsem):
        scale = _D ** -0.5
        pre = [(xa_h, xa_v), (xb_h, xb_v), (wq_h, wq_v), (bwq_h, bwq_v), (wuk_h, wuk_v)]
        pre += [(c_h.at[b], c_v.at[b]) for b in range(_B)]
        pre += [(wuv_h, wuv_v), (bwo_h, bwo_v), (wo_h, wo_v)]
        cps = [pltpu.make_async_copy(s, d, wsem.at[i]) for i, (s, d) in enumerate(pre)]
        for cp in cps[:-1]:
            cp.start()

        def kcp(i, slot):
            return pltpu.make_async_copy(k_h.at[i], k_v.at[slot], ksem.at[slot])

        def vcp(i, slot):
            return pltpu.make_async_copy(v_h.at[i], v_v.at[slot], vsem.at[slot])

        for i in range(nbuf):
            kcp(i, i).start()
            vcp(i, i).start()

        cps[0].wait(); cps[1].wait(); cps[2].wait()
        qa = jnp.dot(xa_v[...], wq_v[...], preferred_element_type=F32)
        for h in range(_H):
            qa_s[h] = qa[:, h * _D:(h + 1) * _D]
        oa_s[...] = jnp.zeros(oa_s.shape, F32)

        cps[3].wait()
        qb = jnp.dot(xb_v[...], bwq_v[...].reshape(_M, _H * _D), preferred_element_type=F32).astype(BF16)
        cps[4].wait()
        wuk = wuk_v[...].reshape(_C, _H * _D)
        for h in range(_H):
            r = lax.dot_general(qb[:, h * _D:(h + 1) * _D], wuk[:, h * _D:(h + 1) * _D], _NT, preferred_element_type=F32)
            for b in range(_B):
                qc_s[b, h:h + 1, :] = r[b:b + 1, :]
        for b in range(_B):
            cps[5 + b].wait()
            c = c_v[b]
            s = lax.dot_general(qc_s[b].astype(BF16), c, _NT, preferred_element_type=F32) * scale
            p = jnp.exp(s - jnp.max(s, axis=-1, keepdims=True))
            l = jnp.sum(p, axis=-1, keepdims=True)
            cc_s[b] = jnp.dot(p.astype(BF16), c, preferred_element_type=F32) / l
        cps[9].wait()
        wuv = wuv_v[...].reshape(_C, _H * _D)
        cps[10].wait()
        ob = jnp.zeros((_B, _M), F32)
        for h in range(_H):
            cch = jnp.concatenate([cc_s[b, h:h + 1, :] for b in range(_B)], axis=0).astype(BF16)
            ctx = jnp.dot(cch, wuv[:, h * _D:(h + 1) * _D], preferred_element_type=F32).astype(BF16)
            ob = ob + lax.dot_general(ctx, bwo_v[h], _NT, preferred_element_type=F32)

        row = lax.broadcasted_iota(jnp.int32, (_B, _D), 0)

        def step(i, carry):
            slot = lax.rem(i, nbuf)
            b = i // _H
            h = lax.rem(i, _H)
            if skip_dma:
                @pl.when(i < nbuf)
                def _():
                    kcp(i, slot).wait()
                    vcp(i, slot).wait()
            else:
                kcp(i, slot).wait()
                vcp(i, slot).wait()
            q = qa_s[h].astype(BF16)
            s = lax.dot_general(q, k_v[slot], _NT, preferred_element_type=F32) * scale
            p = jnp.exp(s - jnp.max(s, axis=-1, keepdims=True))
            l = jnp.sum(p, axis=-1, keepdims=True)
            o = jnp.dot(p.astype(BF16), v_v[slot], preferred_element_type=F32) / l
            oa_s[h] = jnp.where(row == b, o, oa_s[h])

            if not skip_dma:
                @pl.when(i + nbuf < _B * _H)
                def _():
                    kcp(i + nbuf, slot).start()
                    vcp(i + nbuf, slot).start()

            @pl.when(i + nbuf == _B * _H)
            def _():
                cps[-1].start()
            return carry

        lax.fori_loop(0, _B * _H, step, 0)
        oa = jnp.concatenate([oa_s[h] for h in range(_H)], axis=1).astype(BF16)
        cps[-1].wait()
        a = lax.dot_general(oa, wo_v[...], _NT, preferred_element_type=F32)
        o_ref[...] = jnp.concatenate([a, ob], axis=1).astype(o_ref.dtype)

    @jax.jit
    def fn(A_x, A_k_cache, A_v_cache, A_wq, A_wo, B_x, B_c_kv, B_w_q, B_w_uk, B_w_uv, B_w_o):
        out = pl.pallas_call(
            body,
            in_specs=[pl.BlockSpec(memory_space=pl.ANY)] * 11,
            out_specs=pl.BlockSpec(memory_space=pltpu.VMEM),
            out_shape=jax.ShapeDtypeStruct((_B, 2 * _M), BF16),
            scratch_shapes=[
                pltpu.VMEM((_B, _M), BF16), pltpu.VMEM((_B, _M), BF16),
                pltpu.VMEM((_M, _H * _D), BF16), pltpu.VMEM((_M, _H * _D), BF16),
                pltpu.VMEM((_B, _S, _C), BF16), pltpu.VMEM((_M, _H, _D), BF16),
                pltpu.VMEM((_C, _H, _D), BF16), pltpu.VMEM((_C, _H, _D), BF16),
                pltpu.VMEM((_H, _M, _D), BF16),
                pltpu.VMEM((nbuf, _S, _D), BF16), pltpu.VMEM((nbuf, _S, _D), BF16),
                pltpu.VMEM((_H, _B, _D), F32), pltpu.VMEM((_H, _B, _D), F32),
                pltpu.VMEM((_B, _H, _C), F32), pltpu.VMEM((_B, _H, _C), F32),
                pltpu.SemaphoreType.DMA((12,)), pltpu.SemaphoreType.DMA((nbuf,)), pltpu.SemaphoreType.DMA((nbuf,)),
            ],
            compiler_params=pltpu.CompilerParams(vmem_limit_bytes=110 * 2**20),
            name="fused_decode",
        )(A_x.reshape(_B, _M), A_k_cache.reshape(_B * _H, _S, _D), A_v_cache.reshape(_B * _H, _S, _D),
          A_wq, A_wo.T, B_x.reshape(_B, _M), B_c_kv, B_w_q, B_w_uk, B_w_uv, jnp.swapaxes(B_w_o, 1, 2))
        return out.reshape(_B, 1, 2 * _M)
    return fn


@jax.jit
def pallas_concat_heads__mha_block_cached__compressed_kv_cla__decode_kernel(
    A_x, A_k_cache, A_v_cache, A_wq, A_wo, B_x, B_c_kv, B_w_q, B_w_uk, B_w_uv, B_w_o,
):
    return _make()(A_x, A_k_cache, A_v_cache, A_wq, A_wo, B_x, B_c_kv, B_w_q, B_w_uk, B_w_uv, B_w_o)
```

```python
import jax
import jax.numpy as jnp
from jax import lax
import jax.experimental.pallas as pl
import jax.experimental.pallas.tpu as pltpu

_B, _H, _S, _D, _M, _C = 4, 32, 4096, 128, 576, 512
_NT = (((1,), (1,)), ((), ()))
F32, BF16 = jnp.float32, jnp.bfloat16
_G = 8
_MQ = _M // 4


def _make(depth=4, drows=192, nobc=False, first=0, unroll=1, scopes=False):
    names = ["Q", "UK", "C", "UV", "P", "A", "O"]
    counts = [4, 2, 8, 2, 2, _B * _H, 2]
    start = {}
    t0 = 0
    for n, c in zip(names, counts):
        start[n] = (t0, t0 + c)
        t0 += c
    T = t0

    def body(xa_h, k_h, v_h, wq_h, wo_h, xb_h, c_h, bwq_h, wuk_h, wuv_h, bwo_h, o_ref,
             xa_v, xb_v, wq_v, wo_v, c_v, bwq_v, wuk_v, wuv_v, bwo_v, kv_v,
             wt_s, xb_s, qa_s, oa_s, qb_s, t_s, qc_s, m_s, l_s, acc_s, cc_s, ctx_s, out_s, xsem, sems):
        scale = _D ** -0.5

        def streams(name, j):
            if name == "Q":
                return [(wq_h.at[:, pl.ds(pl.multiple_of(j * _G * _D, _G * _D), _G * _D)], wq_v.at[j], 24),
                        (bwq_h.at[j], bwq_v.at[j], 192)]
            if name == "UK":
                return [(wuk_h.at[2 * j + e], wuk_v.at[2 * j + e], 192) for e in range(2)]
            if name == "UV":
                return [(wuv_h.at[2 * j + e], wuv_v.at[2 * j + e], 192) for e in range(2)]
            if name == "C":
                return [(c_h.at[2 * j + e], c_v.at[2 * j + e], 48) for e in range(2)]
            if name == "P":
                return [(bwo_h.at[2 * j + e], bwo_v.at[2 * j + e], 192) for e in range(2)]
            if name == "A":
                slot = lax.rem(j, depth)
                return [(k_h.at[j], kv_v.at[slot, 0], drows), (v_h.at[j], kv_v.at[slot, 1], drows)]
            if name == "O":
                return [(wo_h.at[:, pl.ds(pl.multiple_of((2 * j + e) * _G * _D, _G * _D), _G * _D)], wo_v.at[2 * j + e], 24)
                        for e in range(2)]

        def sem(t, e):
            return sems.at[2 * lax.rem(t, depth) + e]

        def issue(name, j, t):
            st = streams(name, j)
            nfull = st[0][1].shape[0] // st[0][2]

            def piece(i, full):
                for e, (src, dst, r) in enumerate(st):
                    n = r if full else dst.shape[0] - nfull * r
                    if n:
                        off = pl.multiple_of(i * r, r) if full else nfull * r
                        pltpu.make_async_copy(src.at[pl.ds(off, n)], dst.at[pl.ds(off, n)], sem(t, e)).start(priority=e ^ first)

            def loop(i, carry):
                piece(i, True)
                return carry
            lax.fori_loop(0, nfull, loop, 0, unroll=unroll)
            piece(nfull, False)

        def wait(name, j, t, e):
            dst = streams(name, j)[e][1]
            pltpu.make_async_copy(dst, dst, sem(t, e)).wait()

        def comp_q(j, t):
            @pl.when(j == 0)
            def _():
                pltpu.make_async_copy(xa_h, xa_v, xsem.at[0]).wait()
                pltpu.make_async_copy(xb_h, xb_v, xsem.at[1]).wait()
                xb = xb_v[...].astype(F32)
                for i in range(4):
                    xb_s[i] = xb[:, i * _MQ:(i + 1) * _MQ]
                qb_s[...] = jnp.zeros(qb_s.shape, F32)
                oa_s[...] = jnp.zeros(oa_s.shape, F32)
                ctx_s[...] = jnp.zeros(ctx_s.shape, F32)
                out_s[...] = jnp.zeros(out_s.shape, F32)
            wait("Q", j, t, 0)
            wait("Q", j, t, 1)
            qa = jnp.dot(xa_v[...], wq_v[j], preferred_element_type=F32)
            for i in range(_G):
                qa_s[j * _G + i] = qa[:, i * _D:(i + 1) * _D]
            w = bwq_v[j].reshape(_MQ, _H, _D).reshape(_MQ, _H * _D)
            qb_s[...] += jnp.dot(xb_s[j].astype(BF16), w, preferred_element_type=F32)

        def comp_uk(j, t):
            wait("UK", j, t, 0)
            wait("UK", j, t, 1)

            def blk(i, carry):
                wt_s[...] = jnp.swapaxes(wuk_v[i].reshape(_D, _H, _D), 0, 1)
                for h in range(_H):
                    q = qb_s[:, h * _D:(h + 1) * _D].astype(BF16)
                    t_s[h] = lax.dot_general(q, wt_s[h], _NT, preferred_element_type=F32)
                for b in range(_B):
                    qc_s[b, i] = t_s[:, b, :]
                return carry
            lax.fori_loop(2 * j, 2 * j + 2, blk, 0)

        def comp_c(j, t):
            wait("C", j, t, 0)
            wait("C", j, t, 1)
            b = j // 2

            @pl.when(lax.rem(j, 2) == 0)
            def _():
                m_s[...] = jnp.full(m_s.shape, -jnp.inf, F32)
                l_s[...] = jnp.zeros(l_s.shape, F32)
                acc_s[...] = jnp.zeros(acc_s.shape, F32)

            def blk(i, carry):
                c = c_v[i]
                q = jnp.concatenate([qc_s[b, n] for n in range(4)], axis=1).astype(BF16)
                s = lax.dot_general(q, c, _NT, preferred_element_type=F32) * scale
                m_old = m_s[...]
                m_new = jnp.maximum(m_old, jnp.max(s, axis=-1, keepdims=True))
                p = jnp.exp(s - m_new)
                alpha = jnp.exp(m_old - m_new)
                l_s[...] = alpha * l_s[...] + jnp.sum(p, axis=-1, keepdims=True)
                acc_s[...] = alpha * acc_s[...] + jnp.dot(p.astype(BF16), c, preferred_element_type=F32)
                m_s[...] = m_new
                return carry
            lax.fori_loop(2 * j, 2 * j + 2, blk, 0)

            @pl.when(lax.rem(j, 2) == 1)
            def _():
                cc = acc_s[...] / l_s[...]
                for n in range(4):
                    cc_s[n, b] = cc[:, n * _D:(n + 1) * _D]

        def comp_uv(j, t):
            wait("UV", j, t, 0)
            wait("UV", j, t, 1)

            def blk(i, carry):
                wt_s[...] = jnp.swapaxes(wuv_v[i].reshape(_D, _H, _D), 0, 1)
                for h in range(_H):
                    ctx_s[h] += jnp.dot(cc_s[i, :, h, :].astype(BF16), wt_s[h], preferred_element_type=F32)
                return carry
            lax.fori_loop(2 * j, 2 * j + 2, blk, 0)

        def comp_p(j, t):
            wait("P", j, t, 0)
            wait("P", j, t, 1)

            def blk(i, carry):
                acc = out_s[1]
                for n in range(_G):
                    acc += lax.dot_general(ctx_s[i * _G + n].astype(BF16), bwo_v[i, n * _M:(n + 1) * _M, :], _NT,
                                           preferred_element_type=F32)
                out_s[1] = acc
                return carry
            lax.fori_loop(2 * j, 2 * j + 2, blk, 0)

        def comp_a(j, t):
            wait("A", j, t, 0)
            wait("A", j, t, 1)
            slot = lax.rem(j, depth)
            h = lax.rem(j, _H)
            s = lax.dot_general(qa_s[h].astype(BF16), kv_v[slot, 0], _NT, preferred_element_type=F32) * scale
            p = jnp.exp(s - jnp.max(s, axis=-1, keepdims=True))
            l = jnp.sum(p, axis=-1, keepdims=True)
            o = jnp.dot(p.astype(BF16), kv_v[slot, 1], preferred_element_type=F32) / l
            row = lax.broadcasted_iota(jnp.int32, (_B, _D), 0)
            oa_s[h] = jnp.where(row == j // _H, o, oa_s[h])

        def comp_o(j, t):
            for e in range(2):
                wait("O", j, t, e)
                i = 2 * j + e
                oa = jnp.concatenate([oa_s[i * _G + n] for n in range(_G)], axis=1).astype(BF16)
                out_s[0] += lax.dot_general(oa, wo_v[i], _NT, preferred_element_type=F32)

        comp = dict(Q=comp_q, UK=comp_uk, C=comp_c, UV=comp_uv, P=comp_p, A=comp_a, O=comp_o)

        pltpu.make_async_copy(xa_h, xa_v, xsem.at[0]).start()
        pltpu.make_async_copy(xb_h, xb_v, xsem.at[1]).start()

        def scoped(nm, f, *a):
            if scopes:
                with jax.named_scope(nm):
                    f(*a)
            else:
                f(*a)

        def step(t, carry):
            s = t - depth
            for n in names:
                lo, hi = start[n]
                pl.when(jnp.logical_and(s >= lo, s < hi))(lambda n=n, lo=lo: scoped("comp_" + n, comp[n], s - lo, s))
            for n in names:
                lo, hi = start[n]
                pl.when(jnp.logical_and(t >= lo, t < hi))(lambda n=n, lo=lo: scoped("issue_" + n, issue, n, t - lo, t))
            return carry

        lax.fori_loop(0, T + depth, step, 0)
        o_ref[...] = jnp.concatenate([out_s[0], out_s[1]], axis=1).astype(o_ref.dtype)

    @jax.jit
    def fn(A_x, A_k_cache, A_v_cache, A_wq, A_wo, B_x, B_c_kv, B_w_q, B_w_uk, B_w_uv, B_w_o):
        out = pl.pallas_call(
            body,
            in_specs=[pl.BlockSpec(memory_space=pl.ANY)] * 11,
            out_specs=pl.BlockSpec(memory_space=pltpu.VMEM),
            out_shape=jax.ShapeDtypeStruct((_B, 2 * _M), BF16),
            scratch_shapes=[
                pltpu.VMEM((_B, _M), BF16), pltpu.VMEM((_B, _M), BF16),
                pltpu.VMEM((4, _M, _G * _D), BF16), pltpu.VMEM((4, _M, _G * _D), BF16),
                pltpu.VMEM((16, _S // 4, _C), BF16), pltpu.VMEM((4, _MQ * _H, _D), BF16),
                pltpu.VMEM((4, _D * _H, _D), BF16), pltpu.VMEM((4, _D * _H, _D), BF16),
                pltpu.VMEM((4, _G * _M, _D), BF16),
                pltpu.VMEM((depth, 2, _S, _D), BF16),
                pltpu.VMEM((_H, _D, _D), BF16),
                pltpu.VMEM((4, _B, _MQ), F32),
                pltpu.VMEM((_H, _B, _D), F32), pltpu.VMEM((_H, _B, _D), F32),
                pltpu.VMEM((_B, _H * _D), F32), pltpu.VMEM((_H, _B, _D), F32),
                pltpu.VMEM((_B, 4, _H, _D), F32),
                pltpu.VMEM((_H, 1), F32), pltpu.VMEM((_H, 1), F32), pltpu.VMEM((_H, _C), F32),
                pltpu.VMEM((4, _B, _H, _D), F32), pltpu.VMEM((_H, _B, _D), F32),
                pltpu.VMEM((2, _B, _M), F32),
                pltpu.SemaphoreType.DMA((2,)), pltpu.SemaphoreType.DMA((2 * depth,)),
            ],
            compiler_params=pltpu.CompilerParams(vmem_limit_bytes=100 * 2**20, disable_bounds_checks=nobc),
            name="fused_decode",
        )(A_x.reshape(_B, _M), A_k_cache.reshape(_B * _H, _S, _D), A_v_cache.reshape(_B * _H, _S, _D),
          A_wq, A_wo.T, B_x.reshape(_B, _M), B_c_kv.reshape(16, _S // 4, _C), B_w_q.reshape(4, _MQ * _H, _D),
          B_w_uk.reshape(4, _D * _H, _D), B_w_uv.reshape(4, _D * _H, _D),
          jnp.swapaxes(B_w_o, 1, 2).reshape(4, _G * _M, _D))
        return out.reshape(_B, 1, 2 * _M)
    return fn


@jax.jit
def pallas_concat_heads__mha_block_cached__compressed_kv_cla__decode_kernel(
    A_x, A_k_cache, A_v_cache, A_wq, A_wo, B_x, B_c_kv, B_w_q, B_w_uk, B_w_uv, B_w_o,
):
    return _make()(A_x, A_k_cache, A_v_cache, A_wq, A_wo, B_x, B_c_kv, B_w_q, B_w_uk, B_w_uv, B_w_o)
```

```python
import jax
import jax.numpy as jnp
import numpy as np
from jax import lax
import jax.experimental.pallas as pl
import jax.experimental.pallas.tpu as pltpu

_B, _H, _S, _D, _M, _C = 4, 32, 4096, 128, 576, 512
_NT = (((1,), (1,)), ((), ()))
F32, BF16 = jnp.float32, jnp.bfloat16
_G = 8
_NG = _H // _G
_MQ = _M // 4
_KB = 512
_NKB = _S // _KB
_NEG = float(np.finfo(np.float32).min)


def _make(depth=3, nobc=False, first=0, scopes=False, aorder=(0, 1, 2, 3), vskew=0):
    t_w1, t_w2, t_c, t_a = 0, 4, 8, 16
    n_a = _B * _NG * _NKB
    t_w3 = t_a + n_a
    t_end = t_w3 + 4

    def body(xa_h, k_h, v_h, wq_h, wo_h, xb_h, c_h, bwq_h, wuk_h, wuv_h, bwo_h, o_ref,
             xa_v, xb_v, wq_v, wo_v, c_v, bwq_v, wuk_v, wuv_v, bwo_v, k_v, v_v,
             wt_s, xb_s, qa_s, oa_s, ma_s, la_s, aa_s, qb_s, t_s, qc_s, m_s, l_s, acc_s, cc_s, ctx_s, out_s,
             wsem, rsem):
        scale = _D ** -0.5

        def ds(start, size):
            return pl.ds(pl.multiple_of(start, size), size)

        def pair(d):
            return pl.ds(2 * (d % 2), 2)

        def cols(src, dst, j):
            def f(d, p):
                rows = ds((d // 2) * (_MQ // 2) + p * 8, 8)
                return src.at[pair(d), rows, ds(j * _G * _D, _G * _D)], dst.at[j, pair(d), rows]
            return f

        def quarters(src, dst, j, n):
            def f(d, p):
                rows = ds((d // 2) * (src.shape[1] // 2) + (j * n + p) * 64, 64)
                return src.at[pair(d), rows], dst.at[pair(d), rows]
            return f

        def issue(n, streams):
            def cycle(p, carry):
                for d in aorder:
                    for e, (f, sem) in enumerate(streams):
                        pltpu.make_async_copy(*f(d, p), sem).start(priority=e ^ first)
                return carry
            lax.fori_loop(0, n, cycle, 0)

        def wait(buf, sem):
            pltpu.make_async_copy(buf, buf, sem).wait()

        def issue_w1(j):
            issue(9, [(cols(wq_h, wq_v, j), wsem.at[2]), (quarters(bwq_h, bwq_v, j, 9), wsem.at[3])])

        def issue_w2(j):
            issue(8, [(quarters(wuk_h, wuk_v, j, 8), wsem.at[4]), (quarters(wuv_h, wuv_v, j, 8), wsem.at[5])])

        def issue_c(j):
            def half(e):
                def f(d, p):
                    idx = (pl.ds(8 * e + 2 * d, 2), ds((j * 8 + p) * 16, 16))
                    return c_h.at[idx], c_v.at[idx]
                return f
            issue(8, [(half(e), wsem.at[6]) for e in range(2)])

        def issue_a(j):
            slot = lax.rem(j, depth)
            g = lax.div(j, _NKB)
            r0 = lax.rem(j, _NKB) * _KB

            def heads(src, dst):
                def f(d, p):
                    return (src.at[g, pl.ds(2 * d, 2), ds(r0 + p * 64, 64)], dst.at[slot, pl.ds(2 * d, 2), ds(p * 64, 64)])
                return f
            issue(8, [(heads(k_h, k_v), rsem.at[2 * slot]), (heads(v_h, v_v), rsem.at[2 * slot + 1])])

        def issue_w3(j):
            def f(d, p):
                return bwo_h.at[pl.ds(2 * d, 2), j, ds(p * 64, 64)], bwo_v.at[j, pl.ds(2 * d, 2), ds(p * 64, 64)]
            slot = lax.rem(n_a + j, depth)
            issue(9, [(f, rsem.at[2 * slot]), (cols(wo_h, wo_v, j), rsem.at[2 * slot + 1])])

        def comp_q(j):
            @pl.when(j == 0)
            def _():
                wait(xa_v, wsem.at[0])
                wait(xb_v, wsem.at[1])
                xb = xb_v[...].astype(F32)
                for i in range(4):
                    xb_s[i] = xb[:, i * _MQ:(i + 1) * _MQ]
                qb_s[...] = jnp.zeros(qb_s.shape, F32)
                ctx_s[...] = jnp.zeros(ctx_s.shape, F32)
                out_s[...] = jnp.zeros(out_s.shape, F32)
                wait(wq_v, wsem.at[2])
                wait(bwq_v, wsem.at[3])
            qa = jnp.dot(xa_v[...], wq_v[j].reshape(_M, _G * _D), preferred_element_type=F32)
            for i in range(_G):
                t_s[i] = qa[:, i * _D:(i + 1) * _D]
            for b in range(_B):
                qa_s[b * _NG + j] = t_s[:_G, b, :]
            w = bwq_v[j].reshape(_MQ, _H, _D).reshape(_MQ, _H * _D)
            qb_s[...] += jnp.dot(xb_s[j].astype(BF16), w, preferred_element_type=F32)

        def comp_uk(j):
            @pl.when(j == 0)
            def _():
                wait(wuk_v, wsem.at[4])
            wt_s[...] = jnp.swapaxes(wuk_v[j].reshape(_D, _H, _D), 0, 1)
            for h in range(_H):
                q = qb_s[:, h * _D:(h + 1) * _D].astype(BF16)
                t_s[h] = lax.dot_general(q, wt_s[h], _NT, preferred_element_type=F32)
            for b in range(_B):
                qc_s[b, j] = t_s[:, b, :]

        def comp_c(j):
            @pl.when(j == 0)
            def _():
                wait(c_v, wsem.at[6])
            b = lax.div(j, 4)

            @pl.when(lax.rem(j, 4) == 0)
            def _():
                m_s[...] = jnp.full(m_s.shape, _NEG, F32)
                l_s[...] = jnp.zeros(l_s.shape, F32)
                acc_s[...] = jnp.zeros(acc_s.shape, F32)

            c = c_v[j]
            q = jnp.concatenate([qc_s[b, n] for n in range(4)], axis=1).astype(BF16)
            s = lax.dot_general(q, c, _NT, preferred_element_type=F32) * scale
            m_old = m_s[...]
            m_new = jnp.maximum(m_old, jnp.max(s, axis=-1, keepdims=True))
            p = jnp.exp(s - m_new)
            alpha = jnp.exp(m_old - m_new)
            l_s[...] = alpha * l_s[...] + jnp.sum(p, axis=-1, keepdims=True)
            acc_s[...] = alpha * acc_s[...] + jnp.dot(p.astype(BF16), c, preferred_element_type=F32)
            m_s[...] = m_new

            @pl.when(lax.rem(j, 4) == 3)
            def _():
                cc = acc_s[...] / l_s[...]
                for n in range(4):
                    cc_s[n, b] = cc[:, n * _D:(n + 1) * _D]

        def comp_uv(j):
            @pl.when(j == 0)
            def _():
                wait(wuv_v, wsem.at[5])
            wt_s[...] = jnp.swapaxes(wuv_v[j].reshape(_D, _H, _D), 0, 1)
            for h in range(_H):
                ctx_s[h] += jnp.dot(cc_s[j, :, h, :].astype(BF16), wt_s[h], preferred_element_type=F32)

        def comp_a(j):
            slot = lax.rem(j, depth)
            g = lax.div(j, _NKB)

            @pl.when(lax.rem(j, _NKB) == 0)
            def _():
                ma_s[...] = jnp.full(ma_s.shape, _NEG, F32)
                la_s[...] = jnp.zeros(la_s.shape, F32)
                aa_s[...] = jnp.zeros(aa_s.shape, F32)

            wait(k_v.at[slot], rsem.at[2 * slot])
            wait(v_v.at[slot], rsem.at[2 * slot + 1])
            q = qa_s[g].astype(BF16)
            row = lax.broadcasted_iota(jnp.int32, (_G, _KB), 0)
            s = None
            for i in range(_G):
                si = lax.dot_general(q, k_v[slot, i], _NT, preferred_element_type=F32)
                s = si if s is None else jnp.where(row == i, si, s)
            s = s * scale
            m_old = ma_s[...]
            m_new = jnp.maximum(m_old, jnp.max(s, axis=-1, keepdims=True))
            p = jnp.exp(s - m_new)
            alpha = jnp.exp(m_old - m_new)
            la_s[...] = alpha * la_s[...] + jnp.sum(p, axis=-1, keepdims=True)
            ma_s[...] = m_new
            pb = p.astype(BF16)
            row = lax.broadcasted_iota(jnp.int32, (_G, _D), 0)
            o = None
            for i in range(_G):
                oi = jnp.dot(pb, v_v[slot, i], preferred_element_type=F32)
                o = oi if o is None else jnp.where(row == i, oi, o)
            aa_s[...] = alpha * aa_s[...] + o

            @pl.when(lax.rem(j, _NKB) == _NKB - 1)
            def _():
                oa_s[lax.rem(g, _NG), lax.div(g, _NG)] = aa_s[...] / la_s[...]

        def comp_o(j):
            slot = lax.rem(n_a + j, depth)
            wait(bwo_v.at[j], rsem.at[2 * slot])
            acc = out_s[1]
            for n in range(_G):
                acc += lax.dot_general(ctx_s[4 * n + j].astype(BF16), bwo_v[j, n], _NT, preferred_element_type=F32)
            out_s[1] = acc
            oa = jnp.concatenate([oa_s[j, :, n, :] for n in range(_G)], axis=1).astype(BF16)
            wait(wo_v.at[j], rsem.at[2 * slot + 1])
            out_s[0] += lax.dot_general(oa, wo_v[j].reshape(_M, _G * _D), _NT, preferred_element_type=F32)

        table = [
            ("comp_q", comp_q, t_w2 + 2, 4), ("comp_uk", comp_uk, t_c + 2, 4), ("comp_c", comp_c, t_a + 2, 16),
            ("comp_uv", comp_uv, t_a + 18, 4), ("comp_a", comp_a, t_a + depth, n_a), ("comp_o", comp_o, t_w3 + depth, 4),
            ("issue_w1", issue_w1, t_w1, 4), ("issue_w2", issue_w2, t_w2, 4), ("issue_c", issue_c, t_c, 8),
            ("issue_a", issue_a, t_a, n_a), ("issue_w3", issue_w3, t_w3, 4),
        ]

        pltpu.make_async_copy(xa_h, xa_v, wsem.at[0]).start()
        pltpu.make_async_copy(xb_h, xb_v, wsem.at[1]).start()

        def scoped(nm, f, *a):
            if scopes:
                with jax.named_scope(nm):
                    f(*a)
            else:
                f(*a)

        def step(t, carry):
            for nm, f, lo, n in table:
                pl.when(jnp.logical_and(t >= lo, t < lo + n))(lambda nm=nm, f=f, lo=lo: scoped(nm, f, t - lo))
            return carry

        lax.fori_loop(0, t_end + depth, step, 0)
        o_ref[...] = jnp.concatenate([out_s[0], out_s[1]], axis=1).astype(o_ref.dtype)

    @jax.jit
    def fn(A_x, A_k_cache, A_v_cache, A_wq, A_wo, B_x, B_c_kv, B_w_q, B_w_uk, B_w_uv, B_w_o):
        out = pl.pallas_call(
            body,
            in_specs=[pl.BlockSpec(memory_space=pl.ANY)] * 11,
            out_specs=pl.BlockSpec(memory_space=pltpu.VMEM),
            out_shape=jax.ShapeDtypeStruct((_B, 2 * _M), BF16),
            scratch_shapes=[
                pltpu.VMEM((_B, _M), BF16), pltpu.VMEM((_B, _M), BF16),
                pltpu.VMEM((_NG, 4, _MQ, _G * _D), BF16), pltpu.VMEM((_NG, 4, _MQ, _G * _D), BF16),
                pltpu.VMEM((16, _S // 4, _C), BF16), pltpu.VMEM((4, _MQ * _H, _D), BF16),
                pltpu.VMEM((4, _D * _H, _D), BF16), pltpu.VMEM((4, _D * _H, _D), BF16),
                pltpu.VMEM((4, _G, _M, _D), BF16),
                pltpu.VMEM((depth, _G, _KB, _D), BF16), pltpu.VMEM((depth, _G, _KB, _D), BF16),
                pltpu.VMEM((_H, _D, _D), BF16),
                pltpu.VMEM((4, _B, _MQ), F32),
                pltpu.VMEM((_B * _NG, _G, _D), F32), pltpu.VMEM((_NG, _B, _G, _D), F32),
                pltpu.VMEM((_G, 1), F32), pltpu.VMEM((_G, 1), F32), pltpu.VMEM((_G, _D), F32),
                pltpu.VMEM((_B, _H * _D), F32), pltpu.VMEM((_H, _B, _D), F32),
                pltpu.VMEM((_B, 4, _H, _D), F32),
                pltpu.VMEM((_H, 1), F32), pltpu.VMEM((_H, 1), F32), pltpu.VMEM((_H, _C), F32),
                pltpu.VMEM((4, _B, _H, _D), F32), pltpu.VMEM((_H, _B, _D), F32),
                pltpu.VMEM((2, _B, _M), F32),
                pltpu.SemaphoreType.DMA((7,)), pltpu.SemaphoreType.DMA((2 * depth,)),
            ],
            compiler_params=pltpu.CompilerParams(vmem_limit_bytes=100 * 2**20, disable_bounds_checks=nobc),
            name="fused_decode",
        )(A_x.reshape(_B, _M), A_k_cache.reshape(_B * _NG, _G, _S, _D), A_v_cache.reshape(_B * _NG, _G, _S, _D),
          A_wq.reshape(4, _MQ, _H * _D), A_wo.T.reshape(4, _MQ, _H * _D), B_x.reshape(_B, _M),
          B_c_kv.reshape(16, _S // 4, _C), B_w_q.reshape(4, _MQ * _H, _D),
          B_w_uk.reshape(4, _D * _H, _D), B_w_uv.reshape(4, _D * _H, _D),
          jnp.swapaxes(B_w_o, 1, 2).reshape(_G, 4, _M, _D))
        return out.reshape(_B, 1, 2 * _M)
    return fn


@jax.jit
def pallas_concat_heads__mha_block_cached__compressed_kv_cla__decode_kernel(
    A_x, A_k_cache, A_v_cache, A_wq, A_wo, B_x, B_c_kv, B_w_q, B_w_uk, B_w_uv, B_w_o,
):
    return _make()(A_x, A_k_cache, A_v_cache, A_wq, A_wo, B_x, B_c_kv, B_w_q, B_w_uk, B_w_uv, B_w_o)
```

```python
import jax
import jax.numpy as jnp
import numpy as np
from jax import lax
import jax.experimental.pallas as pl
import jax.experimental.pallas.tpu as pltpu

_B, _H, _S, _D, _M, _C = 4, 32, 4096, 128, 576, 512
_NT = (((1,), (1,)), ((), ()))
F32, BF16 = jnp.float32, jnp.bfloat16
_G = 8
_NG = _H // _G
_MQ = _M // 4
_KB = 512
_NKB = _S // _KB
_NEG = float(np.finfo(np.float32).min)
_E = _M % _D


def _make(depth=3, nobc=False, nosc=False, scopes=False, aorder=(0, 1, 2, 3), every=4, last=1):
    t_w2, t_c, t_a = 0, 4, 12
    n_a = _B * _NG * _NKB
    t_w3 = t_a + n_a

    def body(xa_h, k_h, v_h, wq_h, wo_h, xb_h, c_h, bwq_h, wuk_h, wuv_h, bwo_h, o_ref,
             x_v, wq_v, wo_v, c_v, bwq_v, wu_v, bwo_v, kv_v,
             wt_s, xb_s, qa_s, oa_s, ma_s, la_s, aa_s, qb_s, t_s, qc_s, m_s, l_s, acc_s, cc_s, ctx_s, out_s, sems):
        scale = _D ** -0.5

        def ds(start, size):
            return pl.ds(start if isinstance(start, int) else pl.multiple_of(start, size), size)

        def cols(src, dst, j, sem):
            def f(d, p):
                idx = (pl.ds(2 * (d % 2), 2), ds((d // 2) * (_MQ // 2) + p * 8, 8))
                return src.at[(*idx, ds(j * _G * _D, _G * _D))], dst.at[(j, *idx)], sem
            return f

        def rows(src, dst, j, n, sem):
            def f(d, p):
                idx = (pl.ds(2 * (d % 2), 2), ds((d // 2) * (src.shape[1] // 2) + (j * n + p) * 64, 64))
                return src.at[idx], dst.at[idx], sem
            return f

        def issue(n, *streams):
            def cycle(p, carry):
                for d in aorder:
                    for e, f in enumerate(streams):
                        pltpu.make_async_copy(*f(d, p)).start(priority=e)
                return carry
            lax.fori_loop(0, n, cycle, 0)

        def wait(buf, sem):
            pltpu.make_async_copy(buf, buf, sem).wait()

        x_copies = [pltpu.make_async_copy(x_h, x_v.at[e], sems.at[0]) for e, x_h in enumerate((xa_h, xb_h))]

        def issue_w1(j, carry):
            issue(9, cols(wq_h, wq_v, j, sems.at[1]), rows(bwq_h, bwq_v, j, 9, sems.at[2]))
            return carry

        def issue_w2(j):
            issue(8, rows(wuk_h, wu_v.at[0], j, 8, sems.at[depth]), rows(wuv_h, wu_v.at[1], j, 8, sems.at[depth]))

        def issue_c(j):
            def half(e):
                def f(d, p):
                    idx = (pl.ds(8 * e + 2 * d, 2), ds((j * 8 + p) * 16, 16))
                    return c_h.at[idx], c_v.at[idx], sems.at[depth + 1]
                return f
            issue(8, half(0), half(1))

        def issue_a(j):
            slot = lax.rem(j, depth)
            g = lax.div(j, _NKB)
            r0 = lax.rem(j, _NKB) * _KB

            def heads(e, src):
                def f(d, p):
                    return (src.at[g, pl.ds(2 * d, 2), ds(r0 + p * 64, 64)],
                            kv_v.at[slot, e, pl.ds(2 * d, 2), ds(p * 64, 64)], sems.at[slot])
                return f
            issue(8, heads(0, k_h), heads(1, v_h))

        def bwo(j, d, p):
            return bwo_h.at[pl.ds(2 * d, 2), j, ds(p * 64, 64)], bwo_v.at[j, pl.ds(2 * d, 2), ds(p * 64, 64)]

        def issue_w3(j):
            slot = lax.rem(n_a + j, depth)
            issue(9, cols(wo_h, wo_v, j, sems.at[slot]), lambda d, p: (*bwo(j, d, p), sems.at[depth + slot]))

        last_slot = (n_a + _NG - 1) % depth

        def issue_last():
            def f(d, p):
                i = p * 4 + d
                dd = lax.div(i, 9)
                return (*bwo(_NG - 1, dd, i - dd * 9), sems.at[jnp.where(dd < 4 - last, depth + last_slot, 2 * depth)])
            issue(9, cols(wo_h, wo_v, _NG - 1, sems.at[last_slot]), f)

        def comp_q(j):
            @pl.when(j == 0)
            def _():
                for cp in x_copies:
                    cp.wait()
                xb = x_v[1].astype(F32)
                for i in range(4):
                    xb_s[i] = xb[:, i * _MQ:(i + 1) * _MQ]
                qb_s[...] = jnp.zeros(qb_s.shape, F32)
                ctx_s[...] = jnp.zeros(ctx_s.shape, F32)
                out_s[...] = jnp.zeros(out_s.shape, F32)
                wait(wq_v, sems.at[1])
                wait(bwq_v, sems.at[2])
            qa = jnp.dot(x_v[0], wq_v[j].reshape(_M, _G * _D), preferred_element_type=F32)
            for i in range(_G):
                t_s[i] = qa[:, i * _D:(i + 1) * _D]
            for b in range(_B):
                qa_s[b * _NG + j] = t_s[:_G, b, :]
            w = bwq_v[j].reshape(_MQ, _H, _D).reshape(_MQ, _H * _D)
            qb_s[...] += jnp.dot(xb_s[j].astype(BF16), w, preferred_element_type=F32)

        def comp_uk(j):
            @pl.when(j == 0)
            def _():
                wait(wu_v, sems.at[depth])
            wt_s[...] = jnp.swapaxes(wu_v[0, j].reshape(_D, _H, _D), 0, 1)
            for h in range(_H):
                q = qb_s[:, h * _D:(h + 1) * _D].astype(BF16)
                t_s[h] = lax.dot_general(q, wt_s[h], _NT, preferred_element_type=F32)
            for b in range(_B):
                qc_s[b, j] = t_s[:, b, :]

        def comp_c(j):
            @pl.when(j == 0)
            def _():
                wait(c_v, sems.at[depth + 1])
            b = lax.div(j, 4)

            @pl.when(lax.rem(j, 4) == 0)
            def _():
                m_s[...] = jnp.full(m_s.shape, _NEG, F32)
                l_s[...] = jnp.zeros(l_s.shape, F32)
                acc_s[...] = jnp.zeros(acc_s.shape, F32)

            c = c_v[j]
            q = jnp.concatenate([qc_s[b, n] for n in range(4)], axis=1).astype(BF16)
            s = lax.dot_general(q, c, _NT, preferred_element_type=F32) * scale
            m_old = m_s[...]
            m_new = jnp.maximum(m_old, jnp.max(s, axis=-1, keepdims=True))
            p = jnp.exp(s - m_new)
            alpha = jnp.exp(m_old - m_new)
            l_s[...] = alpha * l_s[...] + jnp.sum(p, axis=-1, keepdims=True)
            acc_s[...] = alpha * acc_s[...] + jnp.dot(p.astype(BF16), c, preferred_element_type=F32)
            m_s[...] = m_new

            @pl.when(lax.rem(j, 4) == 3)
            def _():
                cc = acc_s[...] / l_s[...]
                for n in range(4):
                    cc_s[n, b] = cc[:, n * _D:(n + 1) * _D]

        def comp_uv(j):
            wt_s[...] = jnp.swapaxes(wu_v[1, j].reshape(_D, _H, _D), 0, 1)
            for h in range(_H):
                ctx_s[h] += jnp.dot(cc_s[j, :, h, :].astype(BF16), wt_s[h], preferred_element_type=F32)

        def comp_a(j):
            slot = lax.rem(j, depth)
            g = lax.div(j, _NKB)

            @pl.when(lax.rem(j, _NKB) == 0)
            def _():
                ma_s[...] = jnp.full(ma_s.shape, _NEG, F32)
                la_s[...] = jnp.zeros(la_s.shape, F32)
                aa_s[...] = jnp.zeros(aa_s.shape, F32)

            wait(kv_v.at[slot], sems.at[slot])
            q = qa_s[g].astype(BF16)
            row = lax.broadcasted_iota(jnp.int32, (_G, _KB), 0)
            s = None
            for i in range(_G):
                si = lax.dot_general(q, kv_v[slot, 0, i], _NT, preferred_element_type=F32)
                s = si if s is None else jnp.where(row == i, si, s)
            s = s * scale
            m_old = ma_s[...]
            m_new = jnp.maximum(m_old, jnp.max(s, axis=-1, keepdims=True))
            p = jnp.exp(s - m_new)
            alpha = jnp.exp(m_old - m_new)
            la_s[...] = alpha * la_s[...] + jnp.sum(p, axis=-1, keepdims=True)
            ma_s[...] = m_new
            pb = p.astype(BF16)
            row = lax.broadcasted_iota(jnp.int32, (_G, _D), 0)
            o = None
            for i in range(_G):
                oi = jnp.dot(pb, kv_v[slot, 1, i], preferred_element_type=F32)
                o = oi if o is None else jnp.where(row == i, oi, o)
            aa_s[...] = alpha * aa_s[...] + o

            @pl.when(lax.rem(j, _NKB) == _NKB - 1)
            def _():
                oa_s[lax.rem(g, _NG), lax.div(g, _NG)] = aa_s[...] / la_s[...]

        def proj_a(j, sem):
            oa = jnp.concatenate([oa_s[j, :, n, :] for n in range(_G)], axis=1).astype(BF16)
            wait(wo_v.at[j], sem)
            w = wo_v[j].reshape(_M, _G * _D)
            w = jnp.concatenate([w, w[_M - _E:]], axis=0)
            return lax.dot_general(oa, w, _NT, preferred_element_type=F32)

        def proj_b(acc, j, n0, n1, sem):
            ctx = [ctx_s[_NG * n + j].astype(BF16) for n in range(n0, n1)]
            wait(bwo_v.at[j, pl.ds(n0, n1 - n0)], sem)
            for n in range(n0, n1):
                w = bwo_v[j, n]
                w = jnp.concatenate([w[:_E], w], axis=0)
                acc += lax.dot_general(ctx[n - n0], w, _NT, preferred_element_type=F32)
            return acc

        def comp_o(j):
            slot = lax.rem(n_a + j, depth)
            out_s[0] += proj_a(j, sems.at[slot])
            out_s[1] = proj_b(out_s[1], j, 0, _G, sems.at[depth + slot])

        table = [
            ("comp_q", comp_q, t_w2 + 2, 4, 1), ("comp_uk", comp_uk, t_c + 2, 4, 1),
            ("comp_c", comp_c, t_a + 2, 16, every), ("comp_uv", comp_uv, t_a + 2 + 16 * every, 4, every),
            ("comp_a", comp_a, t_a + depth, n_a, 1), ("comp_o", comp_o, t_w3 + depth, _NG - 1, 1),
            ("issue_w2", issue_w2, t_w2, 4, 1), ("issue_c", issue_c, t_c, 8, 1),
            ("issue_a", issue_a, t_a, n_a, 1), ("issue_w3", issue_w3, t_w3, _NG - 1, 1),
            ("issue_last", lambda j: issue_last(), t_w3 + _NG - 1, 1, 1),
        ]

        def scoped(nm, f, *a):
            if scopes:
                with jax.named_scope(nm):
                    return f(*a)
            return f(*a)

        def step(t, carry):
            for nm, f, lo, n, gap in table:
                cond = jnp.logical_and(t >= lo, t < lo + n * gap)
                if gap > 1:
                    cond = jnp.logical_and(cond, lax.rem(t - lo, gap) == 0)
                pl.when(cond)(lambda nm=nm, f=f, lo=lo, gap=gap: scoped(nm, f, lax.div(t - lo, gap)))
            return carry

        lax.fori_loop(0, 4, issue_w1, 0)
        for cp in x_copies:
            cp.start()
        lax.fori_loop(0, t_w3 + depth + _NG - 1, step, 0)

        a = out_s[0] + scoped("comp_la", proj_a, _NG - 1, sems.at[last_slot])
        o_ref[:, :_M - _E] = a[:, :_M - _E].astype(o_ref.dtype)
        b = scoped("comp_lb0", proj_b, out_s[1], _NG - 1, 0, _G - 2 * last, sems.at[depth + last_slot])
        b = scoped("comp_lb1", proj_b, b, _NG - 1, _G - 2 * last, _G, sems.at[2 * depth])
        lane = lax.broadcasted_iota(jnp.int32, (_B, _D), 1)
        seam = jnp.where(lane < _E, a[:, _M - _E:], b[:, :_D])
        o_ref[:, _M - _E:] = jnp.concatenate([seam, b[:, _D:]], axis=1).astype(o_ref.dtype)

    @jax.jit
    def fn(A_x, A_k_cache, A_v_cache, A_wq, A_wo, B_x, B_c_kv, B_w_q, B_w_uk, B_w_uv, B_w_o):
        out = pl.pallas_call(
            body,
            in_specs=[pl.BlockSpec(memory_space=pl.ANY)] * 11,
            out_specs=pl.BlockSpec(memory_space=pltpu.VMEM),
            out_shape=jax.ShapeDtypeStruct((_B, 2 * _M), BF16),
            scratch_shapes=[
                pltpu.VMEM((2, _B, _M), BF16),
                pltpu.VMEM((_NG, 4, _MQ, _G * _D), BF16), pltpu.VMEM((_NG, 4, _MQ, _G * _D), BF16),
                pltpu.VMEM((16, _S // 4, _C), BF16), pltpu.VMEM((4, _MQ * _H, _D), BF16),
                pltpu.VMEM((2, 4, _D * _H, _D), BF16),
                pltpu.VMEM((_NG, _G, _M, _D), BF16),
                pltpu.VMEM((depth, 2, _G, _KB, _D), BF16),
                pltpu.VMEM((_H, _D, _D), BF16),
                pltpu.VMEM((4, _B, _MQ), F32),
                pltpu.VMEM((_B * _NG, _G, _D), F32), pltpu.VMEM((_NG, _B, _G, _D), F32),
                pltpu.VMEM((_G, 1), F32), pltpu.VMEM((_G, 1), F32), pltpu.VMEM((_G, _D), F32),
                pltpu.VMEM((_B, _H * _D), F32), pltpu.VMEM((_H, _B, _D), F32),
                pltpu.VMEM((_B, 4, _H, _D), F32),
                pltpu.VMEM((_H, 1), F32), pltpu.VMEM((_H, 1), F32), pltpu.VMEM((_H, _C), F32),
                pltpu.VMEM((4, _B, _H, _D), F32), pltpu.VMEM((_H, _B, _D), F32),
                pltpu.VMEM((2, _B, _M + _E), F32),
                pltpu.SemaphoreType.DMA((2 * depth + 1,)),
            ],
            compiler_params=pltpu.CompilerParams(vmem_limit_bytes=100 * 2**20, disable_bounds_checks=nobc,
                                                 disable_semaphore_checks=nosc),
            name="fused_decode",
        )(A_x.reshape(_B, _M), A_k_cache.reshape(_B * _NG, _G, _S, _D), A_v_cache.reshape(_B * _NG, _G, _S, _D),
          A_wq.reshape(4, _MQ, _H * _D), A_wo.T.reshape(4, _MQ, _H * _D), B_x.reshape(_B, _M),
          B_c_kv.reshape(16, _S // 4, _C), B_w_q.reshape(4, _MQ * _H, _D),
          B_w_uk.reshape(4, _D * _H, _D), B_w_uv.reshape(4, _D * _H, _D),
          jnp.swapaxes(B_w_o, 1, 2).reshape(_G, _NG, _M, _D))
        return out.reshape(_B, 1, 2 * _M)
    return fn


@jax.jit
def pallas_concat_heads__mha_block_cached__compressed_kv_cla__decode_kernel(
    A_x, A_k_cache, A_v_cache, A_wq, A_wo, B_x, B_c_kv, B_w_q, B_w_uk, B_w_uv, B_w_o,
):
    return _make()(A_x, A_k_cache, A_v_cache, A_wq, A_wo, B_x, B_c_kv, B_w_q, B_w_uk, B_w_uv, B_w_o)
```

```python
import jax
import jax.numpy as jnp
import numpy as np
from jax import lax
import jax.experimental.pallas as pl
import jax.experimental.pallas.tpu as pltpu

_B, _H, _S, _D, _M, _C = 4, 32, 4096, 128, 576, 512
_G = 8
_NG = _H // _G
_KB = 512
_NKB = _S // _KB
_NA = _B * _NG * _NKB
_MQ = _M // 4
_NC = _C // _D
_CB = 4
_SEAM = _M % _D
_DEPTH = 3
_NT = (((1,), (1,)), ((), ()))
_LOWEST = float(np.finfo(np.float32).min)
_F32, _BF16 = jnp.float32, jnp.bfloat16


def _ds(start, size):
    return pl.ds(start if isinstance(start, int) else pl.multiple_of(start, size), size)


def _fetch(cycles, *streams):
    def cycle(p, carry):
        for d in range(4):
            for priority, stream in enumerate(streams):
                pltpu.make_async_copy(*stream(d, p)).start(priority=priority)
        return carry

    lax.fori_loop(0, cycles, cycle, 0)


def _wait(buf, sem):
    pltpu.make_async_copy(buf, buf, sem).wait()


def _column_stream(src, dst, j, sem):
    def stream(d, p):
        idx = (pl.ds(2 * (d % 2), 2), _ds((d // 2) * (_MQ // 2) + p * 8, 8))
        return src.at[(*idx, _ds(j * _G * _D, _G * _D))], dst.at[(j, *idx)], sem

    return stream


def _row_stream(src, dst, first_cycle, sem):
    def stream(d, p):
        row = (d // 2) * (src.shape[1] // 2) + (first_cycle + p) * 64
        idx = (pl.ds(2 * (d % 2), 2), _ds(row, 64))
        return src.at[idx], dst.at[idx], sem

    return stream


def _softmax_init(m_ref, l_ref, acc_ref):
    m_ref[...] = jnp.full(m_ref.shape, _LOWEST, _F32)
    l_ref[...] = jnp.zeros(l_ref.shape, _F32)
    acc_ref[...] = jnp.zeros(acc_ref.shape, _F32)


def _softmax_update(m_ref, l_ref, acc_ref, s, weighted_sum):
    m_old = m_ref[...]
    m_new = jnp.maximum(m_old, jnp.max(s, axis=-1, keepdims=True))
    p = jnp.exp(s - m_new)
    alpha = jnp.exp(m_old - m_new)
    m_ref[...] = m_new
    l_ref[...] = alpha * l_ref[...] + jnp.sum(p, axis=-1, keepdims=True)
    acc_ref[...] = alpha * acc_ref[...] + weighted_sum(p.astype(_BF16))


def _diagonal_rows(product):
    out = product(0)
    row = lax.broadcasted_iota(jnp.int32, out.shape, 0)
    for i in range(1, _G):
        out = jnp.where(row == i, product(i), out)
    return out


def _kernel(
    xa_h, k_h, v_h, wq_h, wo_h, xb_h, c_h, bwq_h, wuk_h, wuv_h, bwo_h, o_ref,
    x_v, kv_v, wq_v, wo_v, c_v, bwq_v, wu_v, bwo_v,
    qa_s, ma_s, la_s, acca_s, oa_s,
    xb_s, qb_s, qc_s, mb_s, lb_s, accb_s, cc_s, ctx_s,
    wt_s, t_s, out_s, sems,
):
    scale = _D**-0.5
    x_copies = [
        pltpu.make_async_copy(x_h, x_v.at[e], sems.at[0])
        for e, x_h in enumerate((xa_h, xb_h))
    ]
    sem_wq, sem_bwq = sems.at[1], sems.at[2]
    sem_wu, sem_c = sems.at[_DEPTH], sems.at[_DEPTH + 1]
    last_slot = (_NA + _NG - 1) % _DEPTH


    def fetch_q_weights(j, carry):
        _fetch(9, _column_stream(wq_h, wq_v, j, sem_wq),
               _row_stream(bwq_h, bwq_v, j * 9, sem_bwq))
        return carry

    def fetch_up_weights(j):
        _fetch(8, _row_stream(wuk_h, wu_v.at[0], j * 8, sem_wu),
               _row_stream(wuv_h, wu_v.at[1], j * 8, sem_wu))

    def fetch_latent(j):
        def half(e):
            def stream(d, p):
                idx = (pl.ds(8 * e + 2 * d, 2), _ds((j * 8 + p) * 16, 16))
                return c_h.at[idx], c_v.at[idx], sem_c

            return stream

        _fetch(8, half(0), half(1))

    def fetch_kv(j):
        slot = lax.rem(j, _DEPTH)
        g = lax.div(j, _NKB)
        key0 = lax.rem(j, _NKB) * _KB

        def cache(e, src):
            def stream(d, p):
                heads = pl.ds(2 * d, 2)
                return (src.at[g, heads, _ds(key0 + p * 64, 64)],
                        kv_v.at[slot, e, heads, _ds(p * 64, 64)], sems.at[slot])

            return stream

        _fetch(8, cache(0, k_h), cache(1, v_h))

    def bwo_piece(j, d, p):
        heads, rows = pl.ds(2 * d, 2), _ds(p * 64, 64)
        return bwo_h.at[heads, j, rows], bwo_v.at[j, heads, rows]

    def fetch_out_weights(j):
        slot = lax.rem(_NA + j, _DEPTH)
        _fetch(9, _column_stream(wo_h, wo_v, j, sems.at[slot]),
               lambda d, p: (*bwo_piece(j, d, p), sems.at[_DEPTH + slot]))

    def fetch_last(_):
        def stream(d, p):
            i = p * 4 + d
            pair = lax.div(i, 9)
            sem = jnp.where(pair < 3, _DEPTH + last_slot, 2 * _DEPTH)
            return *bwo_piece(_NG - 1, pair, i - pair * 9), sems.at[sem]

        _fetch(9, _column_stream(wo_h, wo_v, _NG - 1, sems.at[last_slot]), stream)


    def project_queries(j):
        @pl.when(j == 0)
        def _():
            for copy in x_copies:
                copy.wait()
            xb = x_v[1].astype(_F32)
            for i in range(4):
                xb_s[i] = xb[:, i * _MQ:(i + 1) * _MQ]
            qb_s[...] = jnp.zeros(qb_s.shape, _F32)
            _wait(wq_v, sem_wq)
            _wait(bwq_v, sem_bwq)

        qa = jnp.dot(x_v[0], wq_v[j].reshape(_M, _G * _D), preferred_element_type=_F32)
        for i in range(_G):
            t_s[i] = qa[:, i * _D:(i + 1) * _D]
        for b in range(_B):
            qa_s[b * _NG + j] = t_s[:_G, b, :]
        w = bwq_v[j].reshape(_MQ, _H, _D).reshape(_MQ, _H * _D)
        qb_s[...] += jnp.dot(xb_s[j].astype(_BF16), w, preferred_element_type=_F32)

    def query_to_latent(j):
        @pl.when(j == 0)
        def _():
            _wait(wu_v, sem_wu)

        wt_s[...] = jnp.swapaxes(wu_v[0, j].reshape(_D, _H, _D), 0, 1)
        for h in range(_H):
            q = qb_s[:, h * _D:(h + 1) * _D].astype(_BF16)
            t_s[h] = lax.dot_general(q, wt_s[h], _NT, preferred_element_type=_F32)
        for b in range(_B):
            qc_s[b, j] = t_s[:, b, :]

    def attend_latent(j):
        @pl.when(j == 0)
        def _():
            _wait(c_v, sem_c)

        b = lax.div(j, _CB)
        pl.when(lax.rem(j, _CB) == 0)(lambda: _softmax_init(mb_s, lb_s, accb_s))
        c = c_v[j]
        q = jnp.concatenate([qc_s[b, n] for n in range(_NC)], axis=1).astype(_BF16)
        s = lax.dot_general(q, c, _NT, preferred_element_type=_F32) * scale
        _softmax_update(mb_s, lb_s, accb_s, s,
                        lambda p: jnp.dot(p, c, preferred_element_type=_F32))

        @pl.when(lax.rem(j, _CB) == _CB - 1)
        def _():
            cc = accb_s[...] / lb_s[...]
            for n in range(_NC):
                cc_s[n, b] = cc[:, n * _D:(n + 1) * _D]

    def latent_to_context(j):
        @pl.when(j == 0)
        def _():
            ctx_s[...] = jnp.zeros(ctx_s.shape, _F32)

        wt_s[...] = jnp.swapaxes(wu_v[1, j].reshape(_D, _H, _D), 0, 1)
        for h in range(_H):
            cc = cc_s[j, :, h, :].astype(_BF16)
            ctx_s[h] += jnp.dot(cc, wt_s[h], preferred_element_type=_F32)

    def attend_cache(j):
        slot = lax.rem(j, _DEPTH)
        g = lax.div(j, _NKB)
        pl.when(lax.rem(j, _NKB) == 0)(lambda: _softmax_init(ma_s, la_s, acca_s))
        _wait(kv_v.at[slot], sems.at[slot])
        q = qa_s[g].astype(_BF16)
        s = _diagonal_rows(lambda i: lax.dot_general(
            q, kv_v[slot, 0, i], _NT, preferred_element_type=_F32)) * scale
        _softmax_update(ma_s, la_s, acca_s, s, lambda p: _diagonal_rows(
            lambda i: jnp.dot(p, kv_v[slot, 1, i], preferred_element_type=_F32)))

        @pl.when(lax.rem(j, _NKB) == _NKB - 1)
        def _():
            oa_s[lax.rem(g, _NG), lax.div(g, _NG)] = acca_s[...] / la_s[...]


    def project_a(j, sem):
        o = jnp.concatenate([oa_s[j, :, n, :] for n in range(_G)], axis=1).astype(_BF16)
        _wait(wo_v.at[j], sem)
        w = wo_v[j].reshape(_M, _G * _D)
        w = jnp.concatenate([w, w[_M - _SEAM:]], axis=0)
        return lax.dot_general(o, w, _NT, preferred_element_type=_F32)

    def project_b(acc, j, n0, n1, sem):
        ctx = [ctx_s[_NG * n + j].astype(_BF16) for n in range(n0, n1)]
        _wait(bwo_v.at[j, pl.ds(n0, n1 - n0)], sem)
        for n in range(n0, n1):
            w = bwo_v[j, n]
            w = jnp.concatenate([w[:_SEAM], w], axis=0)
            acc += lax.dot_general(ctx[n - n0], w, _NT, preferred_element_type=_F32)
        return acc

    def project_outputs(j):
        @pl.when(j == 0)
        def _():
            out_s[...] = jnp.zeros(out_s.shape, _F32)

        slot = lax.rem(_NA + j, _DEPTH)
        out_s[0] += project_a(j, sems.at[slot])
        out_s[1] = project_b(out_s[1], j, 0, _G, sems.at[_DEPTH + slot])


    t_c, t_kv = 4, 12
    t_out = t_kv + _NA
    schedule = [
        (project_queries, 2, 4, 1),
        (query_to_latent, t_c + 2, _NC, 1),
        (attend_latent, t_kv + 2, _B * _CB, 4),
        (latent_to_context, t_kv + 2 + _B * _CB * 4, _NC, 4),
        (attend_cache, t_kv + _DEPTH, _NA, 1),
        (project_outputs, t_out + _DEPTH, _NG - 1, 1),
        (fetch_up_weights, 0, t_c, 1),
        (fetch_latent, t_c, t_kv - t_c, 1),
        (fetch_kv, t_kv, _NA, 1),
        (fetch_out_weights, t_out, _NG - 1, 1),
        (fetch_last, t_out + _NG - 1, 1, 1),
    ]

    def step(t, carry):
        for work, first, count, gap in schedule:
            due = jnp.logical_and(t >= first, t < first + count * gap)
            if gap > 1:
                due = jnp.logical_and(due, lax.rem(t, gap) == first % gap)
            pl.when(due)(lambda: work(lax.div(t - first, gap)))
        return carry

    lax.fori_loop(0, 4, fetch_q_weights, 0)
    for copy in x_copies:
        copy.start()
    lax.fori_loop(0, t_out + _DEPTH + _NG - 1, step, 0)

    a = out_s[0] + project_a(_NG - 1, sems.at[last_slot])
    o_ref[:, :_M - _SEAM] = a[:, :_M - _SEAM].astype(o_ref.dtype)
    b = project_b(out_s[1], _NG - 1, 0, _G - 2, sems.at[_DEPTH + last_slot])
    b = project_b(b, _NG - 1, _G - 2, _G, sems.at[2 * _DEPTH])
    lane = lax.broadcasted_iota(jnp.int32, (_B, _D), 1)
    seam = jnp.where(lane < _SEAM, a[:, _M - _SEAM:], b[:, :_D])
    o_ref[:, _M - _SEAM:] = jnp.concatenate([seam, b[:, _D:]], axis=1).astype(o_ref.dtype)


@jax.jit
def pallas_concat_heads__mha_block_cached__compressed_kv_cla__decode_kernel(
    A_x: jax.Array,
    A_k_cache: jax.Array,
    A_v_cache: jax.Array,
    A_wq: jax.Array,
    A_wo: jax.Array,
    B_x: jax.Array,
    B_c_kv: jax.Array,
    B_w_q: jax.Array,
    B_w_uk: jax.Array,
    B_w_uv: jax.Array,
    B_w_o: jax.Array,
):
    vmem = pltpu.VMEM
    out = pl.pallas_call(
        _kernel,
        in_specs=[pl.BlockSpec(memory_space=pl.ANY)] * 11,
        out_specs=pl.BlockSpec(memory_space=vmem),
        out_shape=jax.ShapeDtypeStruct((_B, 2 * _M), _BF16),
        scratch_shapes=[
            vmem((2, _B, _M), _BF16),
            vmem((_DEPTH, 2, _G, _KB, _D), _BF16),
            vmem((_NG, 4, _MQ, _G * _D), _BF16),
            vmem((_NG, 4, _MQ, _G * _D), _BF16),
            vmem((_B * _CB, _S // _CB, _C), _BF16),
            vmem((4, _MQ * _H, _D), _BF16),
            vmem((2, _NC, _D * _H, _D), _BF16),
            vmem((_NG, _G, _M, _D), _BF16),
            vmem((_B * _NG, _G, _D), _F32),
            vmem((_G, 1), _F32),
            vmem((_G, 1), _F32),
            vmem((_G, _D), _F32),
            vmem((_NG, _B, _G, _D), _F32),
            vmem((4, _B, _MQ), _F32),
            vmem((_B, _H * _D), _F32),
            vmem((_B, _NC, _H, _D), _F32),
            vmem((_H, 1), _F32),
            vmem((_H, 1), _F32),
            vmem((_H, _C), _F32),
            vmem((_NC, _B, _H, _D), _F32),
            vmem((_H, _B, _D), _F32),
            vmem((_H, _D, _D), _BF16),
            vmem((_H, _B, _D), _F32),
            vmem((2, _B, _M + _SEAM), _F32),
            pltpu.SemaphoreType.DMA((2 * _DEPTH + 1,)),
        ],
        compiler_params=pltpu.CompilerParams(vmem_limit_bytes=100 * 2**20),
    )(
        A_x.reshape(_B, _M),
        A_k_cache.reshape(_B * _NG, _G, _S, _D),
        A_v_cache.reshape(_B * _NG, _G, _S, _D),
        A_wq.reshape(4, _MQ, _H * _D),
        A_wo.T.reshape(4, _MQ, _H * _D),
        B_x.reshape(_B, _M),
        B_c_kv.reshape(_B * _CB, _S // _CB, _C),
        B_w_q.reshape(4, _MQ * _H, _D),
        B_w_uk.reshape(_NC, _D * _H, _D),
        B_w_uv.reshape(_NC, _D * _H, _D),
        jnp.swapaxes(B_w_o, 1, 2).reshape(_G, _NG, _M, _D),
    )
    return out.reshape(_B, 1, 2 * _M)
```
